```python
import jax
import jax.numpy as jnp

def _softmax(x, axis=-1):
    return jax.nn.softmax(x, axis=axis)

def _gelu(x):
    return jax.nn.gelu(x, approximate=True)

def _silu(x):
    return jax.nn.silu(x)

def _sigmoid(x):
    return jax.nn.sigmoid(x)

def _layernorm(x, axis=-1, eps=1e-05):
    m = jnp.mean(x, axis=axis, keepdims=True)
    v = jnp.var(x, axis=axis, keepdims=True)
    return (x - m) / jnp.sqrt(v + eps)

def _scatter_add(tgt, idx, src, axis=0):
    return tgt.at[idx].add(src)

def _segment_sum(src, seg, n):
    return jax.ops.segment_sum(src, seg, n)

class _Rng:

    def __init__(self, key):
        self._k = key

    def _next(self):
        self._k, sub = jax.random.split(self._k)
        return sub

    def normal(self, shape):
        return jax.random.normal(self._next(), shape, dtype=jnp.bfloat16)

    def randint(self, lo, hi, shape):
        return jax.random.randint(self._next(), shape, lo, hi, dtype=jnp.int32)

    def uniform(self, shape, lo=0.0, hi=1.0):
        return jax.random.uniform(self._next(), shape, jnp.bfloat16, lo, hi)

    def permutation(self, n):
        return jax.random.permutation(self._next(), n)
kernel_name = 'adaLN_cond__spectral_gfnet__geglu_ffn__prompt'

def _fwd_setup_inputs():
    _rng = _Rng(jax.random.key(int.from_bytes(__import__("os").urandom(4), "little")))
    _w = lambda a: (lambda t: t.astype(jnp.bfloat16) if jnp.issubdtype(t.dtype, jnp.floating) else t)(jnp.asarray(a))

    def _A_setup():
        B, S, D = (1, 2048, 512)
        Df = D // 2 + 1
        return {'x': _w((lambda *s: _rng.normal(s) * 0.05)(B, S, D)), 'w_r': _w((lambda *s: _rng.normal(s) * 0.05)(S, Df) * 0.02), 'w_i': _w((lambda *s: _rng.normal(s) * 0.05)(S, Df) * 0.02)}
    _A_in = _A_setup()

    def _B_setup():
        B, S, D, F = (1, 2048, 512, 1792)
        return {'x': _w((lambda *s: _rng.normal(s) * 0.05)(B, S, D)), 'w_gate': _w((lambda *s: _rng.normal(s) * 0.05)(D, F)), 'w_up': _w((lambda *s: _rng.normal(s) * 0.05)(D, F)), 'w_down': _w((lambda *s: _rng.normal(s) * 0.05)(F, D))}
    _B_in = _B_setup()
    return {'A_x': _A_in['x'], 'A_w_r': _A_in['w_r'], 'A_w_i': _A_in['w_i'], 'B_x': _B_in['x'], 'B_w_gate': _B_in['w_gate'], 'B_w_up': _B_in['w_up'], 'B_w_down': _B_in['w_down'], 'c': _w((lambda *s: _rng.normal(s) * 0.05)(1, 512)), 'w_mod': _w((lambda *s: _rng.normal(s) * 0.05)(512, 6 * 512) * 512 ** (-0.5))}

def _fwd_reference(A_x, A_w_r, A_w_i, B_x, B_w_gate, B_w_up, B_w_down, c, w_mod):

    def _A_ref(x, w_r, w_i):
        B, S, D = x.shape
        X = (lambda x, axes=(-2, -1): jnp.fft.rfft2(x.astype(jnp.float32), axes=axes))(x, axes=(-2, -1))
        W = w_r + 1j * w_i
        X = X * W
        y = (lambda x, s, axes=(-2, -1): jnp.fft.irfft2(x, s=s, axes=axes).astype(jnp.bfloat16))(X, (S, D), axes=(-2, -1))
        return y

    def _B_ref(x, w_gate, w_up, w_down):
        return _gelu(x @ w_gate) * (x @ w_up) @ w_down
    x = A_x
    mod = (_silu(c) @ w_mod).reshape(c.shape[0], 6, 1, -1)
    sa, ca, ga, sb, cb, gb = (mod[:, 0].copy(), mod[:, 1].copy(), mod[:, 2].copy(), mod[:, 3].copy(), mod[:, 4].copy(), mod[:, 5].copy())
    h = _layernorm(x, axis=-1) * (1 + ca) + sa
    x = x + ga * _A_ref(h, A_w_r, A_w_i)
    h = _layernorm(x, axis=-1) * (1 + cb) + sb
    x = x + gb * _B_ref(h, B_w_gate, B_w_up, B_w_down)
    return x

def setup_inputs():
    _inp = _fwd_setup_inputs()
    _gk = jax.random.fold_in(jax.random.key(int.from_bytes(__import__("os").urandom(4), "little")), 2 ** 31 - 1)
    _shapes = [[1, 2048, 512]]
    _dtypes = ['bfloat16']
    _gks = jax.random.split(_gk, len(_shapes))
    _gs = [jax.random.normal(k, s, dtype=jnp.dtype(d)) * 0.05 for k, s, d in zip(_gks, _shapes, _dtypes)]
    _inp['grad_out'] = _gs[0]
    return _inp

def reference(A_x, A_w_r, A_w_i, B_w_gate, B_w_up, B_w_down, c, w_mod, B_x, grad_out):
    _const = dict(B_x=B_x)

    def _f(*_d):
        return _fwd_reference(**{'A_x': _d[0], 'A_w_r': _d[1], 'A_w_i': _d[2], 'B_w_gate': _d[3], 'B_w_up': _d[4], 'B_w_down': _d[5], 'c': _d[6], 'w_mod': _d[7], **_const})
    _out, _vjp = jax.vjp(_f, A_x, A_w_r, A_w_i, B_w_gate, B_w_up, B_w_down, c, w_mod)
    _grads = _vjp(grad_out)
    _out0 = jnp.asarray(_out)
    return (_out0, *[jnp.asarray(_g) for _g in _grads])
```

```python
import contextlib
import itertools
import math

import jax
import jax.numpy as jnp
import numpy as np
from jax import lax
import jax.experimental.pallas as pl
import jax.experimental.pallas.tpu as pltpu

S, D, F = 2048, 512, 1792
H = S // 2
FH = F // 2
NJ = FH // 128
R = 128
EPS = 1e-5
SCALE = 2.0 / (S * D)
BF, F32, I32 = jnp.bfloat16, jnp.float32, jnp.int32
NT = (((1,), (1,)), ((), ()))
TN = (((0,), (0,)), ((), ()))
HI16 = -65536
SIGN = -2 ** 31
PITCH = 65


def _dft_constants():
    n = np.arange(256, dtype=np.float64)[:, None]
    m = np.arange(128, dtype=np.float64)[None, :]
    te = 2.0 * np.pi * n * m / 256.0
    fe = np.concatenate([np.cos(te), -np.sin(te)], axis=1)
    fe[:, 128] = (-1.0) ** np.arange(256)
    to = 2.0 * np.pi * n * (2.0 * m + 1.0) / 512.0
    fo = np.concatenate([np.cos(to), -np.sin(to)], axis=1)
    f1 = np.arange(32, dtype=np.float64)[:, None, None]
    f0 = np.arange(64, dtype=np.float64)[None, :, None]
    f0 = np.where(f1 >= 16, 63.0 - f0, f0)
    s0 = np.arange(64, dtype=np.float64)[None, None, :]
    th = 2.0 * np.pi * s0 * (f1 + 32.0 * f0) / 2048.0
    c, s = np.cos(th), np.sin(th)
    mf = np.concatenate([np.concatenate([c, s], axis=2), np.concatenate([-s, c], axis=2)], axis=1)
    return np.stack([fe, fo]).astype(np.float32).astype(BF), mf.astype(np.float32).astype(BF)


_FD, _MF = _dft_constants()


def _dot(a, b, dims=None):
    if dims is None:
        return jnp.dot(a, b, preferred_element_type=F32)
    return lax.dot_general(a, b, dims, preferred_element_type=F32)


def _comb_a(x11, x12, x21, x22):
    return (x11 + x22, x21 + x22, x11, x22, x11 + x12, x21 - x11, x12 - x22)


def _comb_b(x11, x12, x21, x22):
    return (x11 + x22, x11, x12 - x22, x21 - x11, x22, x11 + x12, x21 + x22)


def _comb_c(m):
    return (m[0] + m[3] - m[4] + m[6], m[2] + m[4], m[1] + m[3], m[0] - m[1] + m[2] + m[5])


def _comb_dc(d11, d12, d21, d22):
    return (d11 + d22, d21 - d22, d12 + d22, d11 + d21, d12 - d11, d22, d11)


def _comb_da(d):
    return (d[0] + d[2] + d[4] - d[5], d[4] + d[6], d[1] + d[5], d[0] + d[1] + d[3] - d[6])


def _comb_db(d):
    return (d[0] + d[1] - d[3] + d[5], d[2] + d[5], d[3] + d[6], d[0] - d[2] + d[4] + d[6])


def _geglu(gate, up, dact):
    k0 = math.sqrt(2.0 / math.pi)
    k1 = 0.044715
    g2 = gate * gate
    t = jnp.tanh(gate * (k0 + (k0 * k1) * g2))
    cdf = 0.5 + 0.5 * t
    ge = gate * cdf
    dge = cdf + (gate * (0.5 * k0 + (1.5 * k0 * k1) * g2)) * (1.0 - t * t)
    return ge * up, dact * up * dge, dact * ge


def _twiddle(z, k, n, sign):
    re, im = z
    if k == 0:
        return z
    c, s = math.cos(2.0 * math.pi * k / n), sign * math.sin(2.0 * math.pi * k / n)
    if 4 * k == n:
        return (-im, re) if sign > 0 else (im, -re)
    if (8 * k) % n == 0:
        if c * s > 0:
            return (re - im) * c, (re + im) * c
        return (re + im) * c, (im - re) * c
    return re * c - im * s, re * s + im * c


def _fft(xs, sign):
    n = len(xs)
    if n == 1:
        return xs
    if n == 2:
        (ar, ai), (br, bi) = xs
        return [(ar + br, ai + bi), (ar - br, ai - bi)]
    ev, o1, o3 = _fft(xs[0::2], sign), _fft(xs[1::4], sign), _fft(xs[3::4], sign)
    out = [None] * n
    q = n // 4
    for k in range(q):
        ar, ai = _twiddle(o1[k], k, n, sign)
        br, bi = _twiddle(o3[k], 3 * k, n, sign)
        sr, si, dr, di = ar + br, ai + bi, ar - br, ai - bi
        (er, ei), (fr, fi) = ev[k], ev[k + q]
        out[k] = (er + sr, ei + si)
        out[k + 2 * q] = (er - sr, ei - si)
        plus, minus = (fr - di, fi + dr), (fr + di, fi - dr)
        out[k + q], out[k + 3 * q] = (plus, minus) if sign > 0 else (minus, plus)
    return out


def _weave(*streams):
    done = [0] * len(streams)
    for _ in range(sum(n for _, n in streams)):
        live = [i for i, (_, n) in enumerate(streams) if done[i] < n]
        i = min(live, key=lambda k: (done[k] + 0.5) / streams[k][1])
        next(streams[i][0])
        done[i] += 1
    for gen, _ in streams:
        for _ in gen:
            pass


def _layernorm(x):
    xc = x - jnp.mean(x, axis=-1, keepdims=True)
    rstd = lax.rsqrt(jnp.mean(xc * xc, axis=-1, keepdims=True) + EPS)
    return xc * rstd, rstd


def _layernorm_bwd(dn, n, rstd):
    return rstd * (dn - jnp.mean(dn, axis=-1, keepdims=True) - n * jnp.mean(dn * n, axis=-1, keepdims=True))


def _fold8(v):
    acc = v[0:8]
    for i in range(1, v.shape[0] // 8):
        acc = acc + v[8 * i:8 * i + 8]
    return acc


def _unpack(p):
    return lax.bitcast_convert_type(p << 16, F32), lax.bitcast_convert_type(p & HI16, F32)


def _pack(re, im):
    rb = lax.bitcast_convert_type(re.astype(BF).astype(F32), I32)
    ib = lax.bitcast_convert_type(im.astype(BF).astype(F32), I32)
    return lax.shift_right_logical(rb, 16) | ib


def _reverse64(v):
    row = lax.broadcasted_iota(I32, (8, 128), 0)
    odd, upper = (row & 1) == 1, (row & 2) == 2
    out = []
    for i in range(7, -1, -1):
        t = pltpu.roll(v[8 * i:8 * i + 8], 4, 0)
        t = jnp.where(upper, pltpu.roll(t, 2, 0), pltpu.roll(t, 6, 0))
        out.append(jnp.where(odd, pltpu.roll(t, 1, 0), pltpu.roll(t, 7, 0)))
    return jnp.concatenate(out, axis=0)


def _partner(va, vb, special):
    if special:
        return pltpu.roll(_reverse64(va), 1, 0), _reverse64(vb)
    return vb, va


def _slot(f1):
    return (f1 % 2) * 16 + f1 // 2


(S_MODA, S_MODG, S_MODR, S_FD, S_MF, S_WR, S_WI, S_DWR, S_DWI, S_DMA, S_DMB) = range(11)


def _kernel(c_ref, x_hbm, wr_hbm, wi_hbm, wg_hbm, wu_hbm, wd_hbm, wm_hbm, g_hbm, fd_hbm, mf_hbm,
            out_hbm, dx_hbm, dwr_hbm, dwi_hbm, dwg_hbm, dwu_hbm, dwd_hbm, dc_ref, dwm_hbm,
            xv, gv, wm, wgu, wd, wr, wi, fd, mf, ybuf, xs, wt, av, dx1, stage,
            ah, pt, cb, bgu, bd, dact, q, mod, sums,
            sem, sem_x, sem_g, sem_w, sem_o, sem_dx, sem_dd):
    cp = pltpu.make_async_copy
    scopes = contextlib.ExitStack()

    def phase(name):
        scopes.close()
        if name:
            scopes.enter_context(jax.named_scope(name))

    def rows_of(i, n):
        return pl.ds(i * n if isinstance(i, int) else pl.multiple_of(i * n, n), n)

    def half_rows(i, half, n=R):
        start = half * H + i * n
        return pl.ds(start if isinstance(i, int) else pl.multiple_of(start, n), n)

    def x_copy(i, half):
        return cp(x_hbm.at[half_rows(i, half, 256)], xv.at[half_rows(i, half, 256)], sem_x.at[2 * i + half])

    def g_copy(i, half):
        return cp(g_hbm.at[half_rows(i, half, 256)], gv.at[half_rows(i, half, 256)], sem_g.at[2 * i + half])

    def wd_rows(j, half):
        start = half * FH + j * 128
        return pl.ds(start if isinstance(j, int) else pl.multiple_of(start, 128), 128)

    def wd_copy(j, half):
        return cp(wd_hbm.at[wd_rows(j, half)], wd.at[wd_rows(j, half)], sem_dd.at[2 * j + half])

    def wgu_copy(t):
        src = wg_hbm if t < 2 * NJ else wu_hbm
        return cp(src.at[:, pl.ds(128 * (t % (2 * NJ)), 128)], wgu.at[t], sem_w.at[t])

    def mod_copy(lo, hi, s):
        return cp(wm_hbm.at[:, pl.ds(lo, hi - lo)], wm.at[:, pl.ds(lo, hi - lo)], sem.at[s])

    def dmod_copy(lo, hi, s):
        return cp(wm.at[:, pl.ds(lo, hi - lo)], dwm_hbm.at[:, pl.ds(lo, hi - lo)], sem.at[s])

    def out_copy(i, half):
        return cp(stage.at[half_rows(i, half)], out_hbm.at[half_rows(i, half)], sem_o.at[2 * i + half])

    def dx_copy(i, half):
        return cp(stage.at[half_rows(i, half, 256)], dx_hbm.at[half_rows(i, half, 256)], sem_dx.at[2 * i + half])

    def dwgu_copy(dst, t, half):
        j = t % NJ + NJ * half
        slot = (t // NJ) * 2 * NJ + j
        return cp(wgu.at[slot], dst.at[:, rows_of(j, 128)], sem_w.at[slot])

    def dwd_copy(j, half):
        return cp(wd.at[wd_rows(j, half)], dwd_hbm.at[wd_rows(j, half)], sem_dd.at[2 * j + half])

    in_copies = dict(
        moda=mod_copy(0, 2 * D, S_MODA), modr=mod_copy(2 * D, 5 * D, S_MODR), modg=mod_copy(5 * D, 6 * D, S_MODG),
        fd=cp(fd_hbm, fd, sem.at[S_FD]), mf=cp(mf_hbm, mf, sem.at[S_MF]),
        wr=cp(wr_hbm, wr, sem.at[S_WR]), wi=cp(wi_hbm, wi, sem.at[S_WI]))

    def both(copy, i, wait=False):
        for half in range(2):
            copy(i, half).wait() if wait else copy(i, half).start()

    in_copies["modg"].start()
    both(g_copy, 0)
    both(wd_copy, 0)
    for i in range(1, 4):
        both(g_copy, i)

    phase("s00_start")
    cf = c_ref[...].astype(F32)
    sig = 1.0 / (1.0 + jnp.exp(-cf))
    silu = (cf * sig).astype(BF)
    silu16 = jnp.broadcast_to(silu, (16, D))

    def modulation(k):
        mod[k] = _dot(silu16, wm[:, k * D:(k + 1) * D])[0:8]

    def mod_row(k):
        return mod[k, 0:1, :]

    def model_dft(h_lo, h_hi, i):
        h = jnp.concatenate([h_lo + h_hi, h_lo - h_hi], axis=0)
        lo, hi = h[:, :256], h[:, 256:]
        ev = _dot((lo + hi).astype(BF), fd[0])
        od = _dot((lo - hi).astype(BF), fd[1])
        for k, b in enumerate((2 * i, 2 * i + 1, 16 + 2 * i, 17 + 2 * i)):
            r = slice(64 * k, 64 * k + 64)
            ybuf[b, 0:64, 0:128] = ev[r, :128]
            ybuf[b, 64:128, 0:128] = ev[r, 128:]
            ybuf[b, 0:64, 128:256] = od[r, :128]
            ybuf[b, 64:128, 128:256] = od[r, 128:]

    def model_idft(i):
        def gather(lanes):
            return jnp.concatenate(
                [jnp.concatenate([ybuf[b, 0:64, lanes], ybuf[b, 64:128, lanes]], axis=1)
                 for b in (2 * i, 2 * i + 1, 16 + 2 * i, 17 + 2 * i)], axis=0).astype(BF)
        p = _dot(gather(slice(0, 128)), fd[0], NT)
        o = _dot(gather(slice(128, 256)), fd[1], NT)
        y = jnp.concatenate([p + o, p - o], axis=1)
        return y[:R] + y[R:], y[:R] - y[R:]

    def seq_fft(sign):
        for g in range(8):
            re, im = pl.ds(8 * g, 8), pl.ds(64 + 8 * g, 8)
            for lanes in (slice(0, 128), slice(128, 256)):
                for odd in range(2):
                    z = [(ybuf[16 * odd + b, re, lanes], ybuf[16 * odd + b, im, lanes]) for b in range(16)]
                    if odd and sign < 0:
                        z = [_twiddle(v, b, 32, sign) for b, v in enumerate(z)]
                    z = _fft(z, sign)
                    if odd and sign > 0:
                        z = [_twiddle(v, b, 32, sign) for b, v in enumerate(z)]
                    for b in range(16):
                        ybuf[16 * odd + b, re, lanes] = z[b][0]
                        ybuf[16 * odd + b, im, lanes] = z[b][1]
                    yield

    lane0 = lax.broadcasted_iota(I32, (64, 128), 1) == 0

    def residue(f1):
        return pl.ds(PITCH * f1, 64)

    def residue_octet(f0, a):
        return pl.ds(PITCH * 8 * a + (f0 if a < 2 else 63 - f0), 8, stride=PITCH)

    def bd_prep(js):
        for j in js:
            both(wd_copy, j, wait=True)
            for o in range(0, 128, 32):
                lo, hi = pl.ds(128 * j + o, 32), pl.ds(FH + 128 * j + o, 32)
                parts = _comb_b(wd[lo, 0:256].astype(F32), wd[lo, 256:512].astype(F32),
                                wd[hi, 0:256].astype(F32), wd[hi, 256:512].astype(F32))
                for r in range(7):
                    bd[r, lo, :] = parts[r].astype(BF)

    def cb_prep(i):
        for o in range(0, 256, 32):
            lo, hi = pl.ds(256 * i + o, 32), pl.ds(H + 256 * i + o, 32)
            dlo, dhi = gv[lo, :].astype(F32) * mod_row(5), gv[hi, :].astype(F32) * mod_row(5)
            parts = _comb_dc(dlo[:, :256], dlo[:, 256:], dhi[:, :256], dhi[:, 256:])
            for r in range(7):
                cb[r, lo, :] = parts[r].astype(BF)

    def dact_unit(j):
        prods = []
        for r in range(7):
            prods.append(_dot(cb[r], bd[r, rows_of(j, 128), :], NT))
            yield
        parts = _comb_da(prods)
        for k in range(4):
            dact[j, k] = parts[k].astype(BF)

    in_copies["modg"].wait()
    modulation(5)
    for i in range(4):
        both(g_copy, i, wait=True)
        if i == 1:
            for j in range(1, NJ):
                both(wd_copy, j)
            for name in ("moda", "fd"):
                in_copies[name].start()
            bd_prep([0])
        cb_prep(i)
    phase("s01_u0")
    for i in range(4):
        both(x_copy, i)
    _weave((dact_unit(0), 7))
    bd_prep(range(1, NJ))
    for name in ("wr", "wi", "mf"):
        in_copies[name].start()
    _weave((dact_unit(1), 7))

    phase("s02_p1a")
    in_copies["moda"].wait()
    in_copies["fd"].wait()
    modulation(0)
    modulation(1)
    for i in range(4):
        both(x_copy, i, wait=True)
    in_copies["modr"].start()
    for t in range(4 * NJ):
        wgu_copy(t).start()
    for i in range(H // R):
        h = [_layernorm(xv[half_rows(i, half), :].astype(F32))[0] * (1.0 + mod_row(1)) + mod_row(0)
             for half in range(2)]
        model_dft(h[0], h[1], i)

    phase("s03_p1b")
    _weave((dact_unit(2), 7), (seq_fft(-1), 32))

    phase("s04_wprep")
    in_copies["wr"].wait()
    in_copies["wi"].wait()
    in_copies["mf"].wait()

    def filter_prep():
        for t in range(16):
            cols = slice(128 * t, 128 * t + 128)
            r32 = pltpu.bitcast(wr[0:256, cols], I32)
            i32 = pltpu.bitcast(wi[0:256, cols], I32)
            nyq = _pack(wr[256:257, cols].astype(F32), wi[256:257, cols].astype(F32))
            tiles = ((r32 & 0xFFFF) | (i32 << 16), lax.shift_right_logical(r32, 16) | (i32 & HI16),
                     jnp.broadcast_to(nyq, (128, 128)))
            for k, tile in enumerate(tiles):
                tile = tile.T
                for v in range(16):
                    wt[k, residue_octet(4 * t + v // 4, v % 4), :] = tile[8 * v:8 * v + 8]
            yield
        for p in range(16):
            f1s = (p, 32 - p) if p else (0, 16)
            w0, wn = [wt[0, residue(f1), :] for f1 in f1s], [wt[2, residue(f1), :] for f1 in f1s]
            w0m, wnm = _partner(w0[0], w0[1], p == 0), _partner(wn[0], wn[1], p == 0)
            for k, f1 in enumerate(f1s):
                if k == 0 or p == 0:
                    (ar, ai), (br, bi) = _unpack(w0[k]), _unpack(w0m[k])
                    (cr, ci), (dr, di) = _unpack(wn[k]), _unpack(wnm[k])
                    s0r, s0i, snr, sni = ar + br, ai - bi, cr + dr, ci - di
                    alpha = _pack(0.25 * (s0r + snr), 0.25 * (s0i + sni))
                    beta = _pack(0.25 * (s0r - snr), 0.25 * (s0i - sni))
                else:
                    alpha, beta = alpha ^ SIGN, beta ^ SIGN
                wt[0, residue(f1), :] = jnp.where(lane0, alpha, w0[k])
                wt[2, residue(f1), :] = jnp.where(lane0, beta, 0)
            yield
    _weave((dact_unit(3), 7), (filter_prep(), 32))

    phase("s05_p1c")

    def spectrum(p, special):
        f1s = (0, 16) if special else (p, 32 - p)
        z = [_dot(mf[f1], ybuf[_slot(f1)].astype(BF)) for f1 in f1s]
        mr = _partner(z[0][0:64, 0:128], z[1][0:64, 0:128], special)
        mi = _partner(z[0][64:128, 0:128], z[1][64:128, 0:128], special)
        return f1s, z, mr, mi

    def filter_and_invert(f1, z, mr, mi, conj):
        er, ei, orr, oi = z[0:64, 0:128], z[64:128, 0:128], z[0:64, 128:256], z[64:128, 128:256]
        (ar, ai), (wr_, wi_), (br, bi) = [_unpack(wt[k, residue(f1), :]) for k in range(3)]
        if conj:
            pe = (ar * er + ai * ei + (br * mr - bi * mi), ar * ei - ai * er - (br * mi + bi * mr))
            po = (wr_ * orr + wi_ * oi, wr_ * oi - wi_ * orr)
        else:
            pe = (ar * er - ai * ei + (br * mr + bi * mi), ar * ei + ai * er + (bi * mr - br * mi))
            po = (wr_ * orr - wi_ * oi, wr_ * oi + wi_ * orr)
        prod = jnp.concatenate([jnp.concatenate([pe[0], po[0]], axis=1),
                                jnp.concatenate([pe[1], po[1]], axis=1)], axis=0)
        ybuf[_slot(f1)] = _dot(mf[f1], prod.astype(BF), TN)

    for p in range(16):
        f1s, z, mr, mi = spectrum(p, p == 0)
        for k, f1 in enumerate(f1s):
            er, ei = z[k][0:64, 0:128], z[k][64:128, 0:128]
            xs[f1, 0:64, 0:128] = jnp.where(lane0, 0.125 * (er + mr[k]), er).astype(BF)
            xs[f1, 64:128, 0:128] = jnp.where(lane0, 0.125 * (ei - mi[k]), ei).astype(BF)
            xs[f1, :, 128:256] = z[k][:, 128:256].astype(BF)
            xs[f1, 0:64, 256:384] = (0.125 * (er - mr[k])).astype(BF)
            xs[f1, 64:128, 256:384] = (0.125 * (ei + mi[k])).astype(BF)
            filter_and_invert(f1, z[k], mr[k], mi[k], False)

    phase("s06_p1d")
    _weave((dact_unit(4), 7), (seq_fft(1), 32))

    phase("s07_bgu")
    in_copies["modr"].wait()
    for t in range(4 * NJ):
        wgu_copy(t).wait()
    for k in (2, 3, 4):
        modulation(k)

    def bgu_prep():
        for t in range(2 * NJ):
            lo = (t // NJ) * 2 * NJ + t % NJ
            for o in range(0, 256, 64):
                a, b = slice(o, o + 64), slice(256 + o, 256 + o + 64)
                parts = _comb_b(wgu[lo, a].astype(F32), wgu[lo + NJ, a].astype(F32),
                                wgu[lo, b].astype(F32), wgu[lo + NJ, b].astype(F32))
                for r in range(7):
                    bgu[t, r, a] = parts[r].astype(BF)
            yield
    _weave((dact_unit(5), 7), (bgu_prep(), 2 * NJ))

    phase("s08_stage0")

    def residual1(rows):
        return xv[rows, :].astype(F32) + (SCALE * mod_row(2)) * av[rows, :].astype(F32)

    def stage0():
        for i in range(H // R):
            a = model_idft(i)
            yield
            h = []
            for half in range(2):
                av[half_rows(i, half), :] = a[half].astype(BF)
                n, _ = _layernorm(residual1(half_rows(i, half)))
                h.append(n * (1.0 + mod_row(4)) + mod_row(3))
            parts = _comb_a(h[0][:, :256], h[0][:, 256:], h[1][:, :256], h[1][:, 256:])
            for r in range(7):
                ah[r, rows_of(i, R), :] = parts[r].astype(BF)
            yield
    _weave((dact_unit(6), 7), (stage0(), 16))

    sums[...] = jnp.zeros(sums.shape, F32)

    def gate_up(i, j):
        return [_dot(ah[r, rows_of(i, R), :], jnp.concatenate([bgu[j, r], bgu[NJ + j, r]], axis=1))
                for r in range(7)]

    def geglu_chunk(i, j, prods):
        rows = rows_of(i, R)
        res = [_geglu(gu[:, :128], gu[:, 128:], dact[j, k, rows, :].astype(F32))
               for k, gu in enumerate(_comb_c(prods))]
        for t, parts in ((2 * NJ + j, _comb_a(*[v[0] for v in res])),
                         (j, _comb_dc(*[v[1] for v in res])),
                         (NJ + j, _comb_dc(*[v[2] for v in res]))):
            for r in range(7):
                q[t, r, rows, :] = parts[r].astype(BF)

    def down_products(i, r):
        rows = rows_of(i, R)
        down = _dot(jnp.concatenate([q[2 * NJ + j, r, rows, :] for j in range(NJ)], axis=1), bd[r])
        dh = _dot(jnp.concatenate([q[t, r, rows, :] for t in range(2 * NJ)], axis=1),
                  jnp.concatenate([bgu[t, r] for t in range(2 * NJ)], axis=1), NT)
        return down, dh

    def ffn_finish(i, prods):
        b = _comb_c([v[0] for v in prods])
        dh = _comb_da([v[1] for v in prods])
        for half in range(2):
            rows = half_rows(i, half)
            bh = jnp.concatenate([b[2 * half], b[2 * half + 1]], axis=1)
            stage[rows, :] = (residual1(rows) + mod_row(5) * bh).astype(BF)
            sums[5] += _fold8(gv[rows, :].astype(F32) * bh)
            dx1[rows, :] = jnp.concatenate([dh[2 * half], dh[2 * half + 1]], axis=1)
            out_copy(i, half).start()

    def ffn_step(i, _):
        prods = gate_up(i, 0)
        for j in range(NJ):
            nxt = gate_up(i, j + 1) if j + 1 < NJ else None
            geglu_chunk(i, j, prods)
            prods = nxt
        tail = []
        for r in range(7):
            tail.append(down_products(i, r))
            pt[0, r, i] = ah[r, rows_of(i, R), :].T
            pt[1, r, i] = cb[r, rows_of(i, R), :].T
        ffn_finish(i, tail)
    phase("s11_ffn")
    lax.fori_loop(0, H // R, ffn_step, None)

    def wgrad(side, t):
        prods = []
        for r in range(7):
            prods.append(_dot(jnp.concatenate([pt[side, r, i] for i in range(H // R)], axis=1), q[t, r]))
            yield
        return _comb_db(prods)

    def wgrad_gate_up(t):
        d11, d12, d21, d22 = yield from wgrad(0, t)
        lo = (t // NJ) * 2 * NJ + t % NJ
        wgu[lo, 0:256] = d11.astype(BF)
        wgu[lo + NJ, 0:256] = d12.astype(BF)
        wgu[lo, 256:512] = d21.astype(BF)
        wgu[lo + NJ, 256:512] = d22.astype(BF)

    def wgrad_gate_up_send(t):
        for half in range(2):
            if isinstance(t, int):
                dwgu_copy(dwg_hbm if t < NJ else dwu_hbm, t, half).start()
                continue

            @pl.when(t < NJ)
            def _():
                dwgu_copy(dwg_hbm, t, half).start()

            @pl.when(t >= NJ)
            def _():
                dwgu_copy(dwu_hbm, t, half).start()

    def wgrad_down(j):
        d11, d12, d21, d22 = yield from wgrad(1, 2 * NJ + j)
        lo, hi = wd_rows(j, 0), wd_rows(j, 1)
        wd[lo, 0:256] = d11.T.astype(BF)
        wd[lo, 256:512] = d12.T.astype(BF)
        wd[hi, 0:256] = d21.T.astype(BF)
        wd[hi, 256:512] = d22.T.astype(BF)
        both(dwd_copy, j)

    phase("s13_stagec")
    def stage_c_rows(i):
        da = []
        for half in range(2):
            rows = half_rows(i, half)
            n, rstd = _layernorm(residual1(rows))
            yield
            dh = dx1[rows, :]
            sums[3] += _fold8(dh)
            sums[4] += _fold8(dh * n)
            d = gv[rows, :].astype(F32) + _layernorm_bwd(dh * (1.0 + mod_row(4)), n, rstd)
            dx1[rows, :] = d
            sums[2] += _fold8(d * av[rows, :].astype(F32))
            da.append(d * (SCALE * mod_row(2)))
            yield
        model_dft(da[0], da[1], i)
        yield

    def stage_c(i, _):
        _weave((wgrad_gate_up(i), 7), (stage_c_rows(i), 5))
        wgrad_gate_up_send(i)
    lax.fori_loop(0, 8, stage_c, None)

    silu_col = jnp.broadcast_to(silu.astype(F32), (128, D)).T

    def modulation_bwd(ks):
        acc = jnp.zeros((16, D), F32)
        for k in ks:
            dm = jnp.sum(sums[k], axis=0, keepdims=True) * (SCALE if k == 2 else 1.0)
            hi = dm.astype(BF)
            lo = (dm - hi.astype(F32)).astype(BF)
            row = lax.broadcasted_iota(I32, (16, D), 0)
            lhs = jnp.where(row == 0, hi.astype(F32), jnp.where(row == 1, lo.astype(F32), 0.0)).astype(BF)
            acc = acc + _dot(lhs, wm[:, k * D:(k + 1) * D], NT)
            for t in range(D // 128):
                cols = slice(k * D + 128 * t, k * D + 128 * t + 128)
                wm[:, cols] = (silu_col * dm[:, 128 * t:128 * t + 128]).astype(BF)
        return acc[0:1] + acc[1:2]

    phase("s14_p3b")
    _weave((wgrad_gate_up(8), 7), (seq_fft(-1), 32))
    wgrad_gate_up_send(8)

    phase("s15_p3c")

    def p3c_pairs(ps, special=False):
        for p in ps:
            f1s, z, mr, mi = spectrum(p, special)
            yield
            for k, f1 in enumerate(f1s):
                filter_and_invert(f1, z[k], mr[k], mi[k], True)
                er, ei = z[k][0:64, 0:128], z[k][64:128, 0:128]
                grads = ((jnp.where(lane0, er + mr[k], er), jnp.where(lane0, ei - mi[k], ei)),
                         (z[k][0:64, 128:256], z[k][64:128, 128:256]),
                         (er - mr[k], ei + mi[k]))
                for t, (gr, gi) in enumerate(grads):
                    xr = xs[f1, 0:64, 128 * t:128 * t + 128].astype(F32)
                    xi = xs[f1, 64:128, 128 * t:128 * t + 128].astype(F32)
                    wt[t, residue(f1), :] = _pack(gr * xr + gi * xi, gi * xr - gr * xi)
                yield

    def p3c(i, _):
        _weave((wgrad_gate_up(9 + i), 7), (p3c_pairs([1 + 5 * i + u for u in range(5)]), 15))
        wgrad_gate_up_send(9 + i)
    lax.fori_loop(0, 3, p3c, None)
    _weave((wgrad_gate_up(12), 7), (p3c_pairs([0], True), 3))
    wgrad_gate_up_send(12)

    phase("s16_p3d")
    _weave((wgrad_gate_up(13), 7), (seq_fft(1), 32))
    wgrad_gate_up_send(13)

    phase("s17_dw")

    def filter_grad_out():
        for t in range(16):
            cols = slice(128 * t, 128 * t + 128)
            ev, od, nyq = [
                jnp.concatenate([wt[k, residue_octet(4 * t + v // 4, v % 4), :] for v in range(16)], axis=0).T
                for k in range(3)]
            wr[0:256, cols] = pltpu.bitcast((ev & 0xFFFF) | (od << 16), BF)
            wi[0:256, cols] = pltpu.bitcast(lax.shift_right_logical(ev, 16) | (od & HI16), BF)
            nr, ni = _unpack(nyq[0:1])
            wr[256:257, cols] = nr.astype(BF)
            wi[256:257, cols] = ni.astype(BF)
            yield
    _weave((wgrad_down(0), 7), (filter_grad_out(), 16))
    dwr_copy, dwi_copy = cp(wr, dwr_hbm, sem.at[S_DWR]), cp(wi, dwi_hbm, sem.at[S_DWI])
    dwr_copy.start()
    dwi_copy.start()
    for i in range(H // R):
        both(out_copy, i, wait=True)

    phase("s18_p3e")

    def p3e_rows(i):
        dhs = model_idft(i)
        yield
        for half in range(2):
            rows, dh = half_rows(i, half), dhs[half]
            n, rstd = _layernorm(xv[rows, :].astype(F32))
            sums[0] += _fold8(dh)
            sums[1] += _fold8(dh * n)
            stage[rows, :] = (dx1[rows, :] + _layernorm_bwd(dh * (1.0 + mod_row(1)), n, rstd)).astype(BF)
            yield

    def p3e(i, _):
        _weave((wgrad_down(1 + i), 7), (itertools.chain(p3e_rows(2 * i), p3e_rows(2 * i + 1)), 6))
        both(dx_copy, i)
    lax.fori_loop(0, 4, p3e, None)

    phase("s19_tail")
    dsilu = modulation_bwd(range(6))
    dmod_copy(0, 6 * D, S_DMA).start()
    dc_ref[...] = (dsilu * (sig * (1.0 + cf * (1.0 - sig)))).astype(dc_ref.dtype)
    _weave((wgrad_down(5), 7))
    _weave((wgrad_down(6), 7))

    phase("s20_wait")
    for t in range(2 * NJ):
        for half in range(2):
            dwgu_copy(dwg_hbm if t < NJ else dwu_hbm, t, half).wait()
    dwr_copy.wait()
    dwi_copy.wait()
    for i in range(4):
        both(dx_copy, i, wait=True)
    dmod_copy(0, 6 * D, S_DMA).wait()
    for j in range(NJ):
        both(dwd_copy, j, wait=True)
    phase(None)


@jax.jit
def pallas_adaLN_cond__spectral_gfnet__geglu_ffn__prompt_kernel(
    A_x: jax.Array,
    A_w_r: jax.Array,
    A_w_i: jax.Array,
    B_x: jax.Array,
    B_w_gate: jax.Array,
    B_w_up: jax.Array,
    B_w_down: jax.Array,
    c: jax.Array,
    w_mod: jax.Array,
    grad_out: jax.Array,
):
    del B_x
    kf = D // 2 + 1
    hbm = pl.BlockSpec(memory_space=pltpu.MemorySpace.HBM)
    vmem = pl.BlockSpec(memory_space=pltpu.MemorySpace.VMEM)
    sds = jax.ShapeDtypeStruct
    dma = pltpu.SemaphoreType.DMA
    out, dx, dwr, dwi, dwg, dwu, dwd, dc, dwm = pl.pallas_call(
        _kernel,
        in_specs=[vmem] + [hbm] * 10,
        out_specs=[hbm] * 7 + [vmem, hbm],
        out_shape=[sds((S, D), BF), sds((S, D), BF), sds((kf, S), BF), sds((kf, S), BF),
                   sds((D, F), BF), sds((D, F), BF), sds((F, D), BF), sds((1, D), BF), sds((D, 6 * D), BF)],
        scratch_shapes=[
            pltpu.VMEM((S, D), BF),
            pltpu.VMEM((S, D), BF),
            pltpu.VMEM((D, 6 * D), BF),
            pltpu.VMEM((4 * NJ, D, 128), BF),
            pltpu.VMEM((F, D), BF),
            pltpu.VMEM((kf, S), BF),
            pltpu.VMEM((kf, S), BF),
            pltpu.VMEM((2, 256, 256), BF),
            pltpu.VMEM((32, 128, 128), BF),
            pltpu.VMEM((32, 128, 256), F32),
            pltpu.VMEM((32, 128, 384), BF),
            pltpu.VMEM((3, 32 * PITCH, 128), I32),
            pltpu.VMEM((S, D), BF),
            pltpu.VMEM((S, D), F32),
            pltpu.VMEM((S, D), BF),
            pltpu.VMEM((7, H, 256), BF),
            pltpu.VMEM((2, 7, H // R, 256, R), BF),
            pltpu.VMEM((7, H, 256), BF),
            pltpu.VMEM((2 * NJ, 7, 256, 128), BF),
            pltpu.VMEM((7, FH, 256), BF),
            pltpu.VMEM((NJ, 4, H, 128), BF),
            pltpu.VMEM((3 * NJ, 7, H, 128), BF),
            pltpu.VMEM((6, 8, D), F32),
            pltpu.VMEM((6, 8, D), F32),
            dma((11,)), dma((8,)), dma((8,)), dma((4 * NJ,)), dma((2 * H // R,)), dma((8,)), dma((2 * NJ,)),
        ],
        compiler_params=pltpu.CompilerParams(vmem_limit_bytes=126 * 1024 * 1024),
    )(c, A_x.reshape(S, D), A_w_r.T, A_w_i.T, B_w_gate, B_w_up, B_w_down, w_mod,
      grad_out.reshape(S, D), _FD, _MF)
    return (out.reshape(1, S, D), dx.reshape(1, S, D), dwr.T, dwi.T, dwg, dwu, dwd, dc, dwm)
```

```python
import contextlib
import itertools
import math

import jax
import jax.numpy as jnp
import numpy as np
from jax import lax
import jax.experimental.pallas as pl
import jax.experimental.pallas.tpu as pltpu

S, D, F = 2048, 512, 1792
H = S // 2
FH = F // 2
NJ = FH // 128
R = 128
EPS = 1e-5
SCALE = 2.0 / (S * D)
BF, F32, I32 = jnp.bfloat16, jnp.float32, jnp.int32
NT = (((1,), (1,)), ((), ()))
HI16 = -65536
SIGN = -2 ** 31
PITCH = 65


def _pack_rows(a):
    bits = a.astype(np.float32).astype(BF).view(np.uint16).astype(np.uint32)
    return (bits[..., 0::2, :] | (bits[..., 1::2, :] << 16)).view(np.int32)


def _dft_constants():
    n = np.arange(256, dtype=np.float64)[:, None]
    m = np.arange(128, dtype=np.float64)[None, :]
    t0 = (2.0 * np.pi * n * m / 128.0)[:128, :64]
    t2 = (2.0 * np.pi * n * (2.0 * m + 1.0) / 256.0)[:128, :64]
    fe = np.zeros((256, 256))
    fe[:128] = np.concatenate([np.cos(t0), -np.sin(t0), -np.sin(t2), np.cos(t2)], axis=1)
    fe[:128, 64] = (-1.0) ** np.arange(128)
    to = 2.0 * np.pi * n * (2.0 * m + 1.0) / 512.0
    fo = np.concatenate([np.cos(to), -np.sin(to)], axis=1)
    co, so = np.cos(to[:128]), np.sin(to[:128]) * (-1.0) ** m
    fo3 = np.block([[co, co + so], [so - co, np.zeros_like(co)]])
    f1 = np.arange(32, dtype=np.float64)[:, None, None]
    f0 = np.arange(64, dtype=np.float64)[None, :, None]
    f0 = np.where(f1 >= 16, 63.0 - f0, f0)
    s0 = np.arange(64, dtype=np.float64)[None, None, :]
    th = 2.0 * np.pi * s0 * (f1 + 32.0 * f0) / 2048.0
    c, s = np.cos(th), np.sin(th)
    mf = np.concatenate([np.concatenate([c, s], axis=2), np.concatenate([-s, c], axis=2)], axis=1)
    return _pack_rows(np.stack([fe, fo, fo3])), _pack_rows(np.stack([mf, mf.transpose(0, 2, 1)]))


_FD, _MF = _dft_constants()


class _Packed:
    def __init__(self, ref):
        self.ref, self.lead = ref, len(ref.shape) - 2

    def _index(self, idx):
        idx = idx if isinstance(idx, tuple) else (idx,)
        if len(idx) <= self.lead:
            return idx
        rows = idx[self.lead]
        if isinstance(rows, slice):
            rows = rows if rows.start is None else slice(rows.start // 2, rows.stop // 2)
        elif isinstance(rows.start, int):
            rows = pl.ds(rows.start // 2, rows.size // 2)
        else:
            rows = pl.ds(pl.multiple_of(rows.start >> 1, rows.size // 2), rows.size // 2)
        return idx[:self.lead] + (rows,) + idx[self.lead + 1:]

    def __getitem__(self, idx):
        return pltpu.bitcast(self.ref[self._index(idx)], BF)

    def __setitem__(self, idx, value):
        self.ref[self._index(idx)] = value if value.dtype == I32 else pltpu.bitcast(value, I32)


def _packed(*shape):
    return pltpu.VMEM(shape[:-2] + (shape[-2] // 2, shape[-1]), I32)


def _dot(a, b, dims=None):
    if dims is None:
        return jnp.dot(a, b, preferred_element_type=F32)
    return lax.dot_general(a, b, dims, preferred_element_type=F32)


def _comb_a(x11, x12, x21, x22):
    return (x11 + x22, x21 + x22, x11, x22, x11 + x12, x21 - x11, x12 - x22)


def _comb_b(x11, x12, x21, x22):
    return (x11 + x22, x11, x12 - x22, x21 - x11, x22, x11 + x12, x21 + x22)


def _comb_c(m):
    return (m[0] + m[3] - m[4] + m[6], m[2] + m[4], m[1] + m[3], m[0] - m[1] + m[2] + m[5])


def _comb_dc(d11, d12, d21, d22):
    return (d11 + d22, d21 - d22, d12 + d22, d11 + d21, d12 - d11, d22, d11)


def _comb_da(d):
    return (d[0] + d[2] + d[4] - d[5], d[4] + d[6], d[1] + d[5], d[0] + d[1] + d[3] - d[6])


def _geglu(gate, up, dact):
    k0 = math.sqrt(2.0 / math.pi)
    k1 = 0.044715
    g2 = gate * gate
    t = jnp.tanh(gate * (k0 + (k0 * k1) * g2))
    cdf = 0.5 + 0.5 * t
    ge = gate * cdf
    dge = cdf + (gate * (0.5 * k0 + (1.5 * k0 * k1) * g2)) * (1.0 - t * t)
    return ge * up, dact * up * dge, dact * ge


def _twiddle(z, k, n, sign):
    re, im = z
    if k == 0:
        return z
    c, s = math.cos(2.0 * math.pi * k / n), sign * math.sin(2.0 * math.pi * k / n)
    if 4 * k == n:
        return (-im, re) if sign > 0 else (im, -re)
    if (8 * k) % n == 0:
        if c * s > 0:
            return (re - im) * c, (re + im) * c
        return (re + im) * c, (im - re) * c
    return re * c - im * s, re * s + im * c


def _fft_merge(ev, o1, o3, k, sign):
    q = len(o1)
    ar, ai = _twiddle(o1[k], k, 4 * q, sign)
    br, bi = _twiddle(o3[k], 3 * k, 4 * q, sign)
    sr, si, dr, di = ar + br, ai + bi, ar - br, ai - bi
    (er, ei), (fr, fi) = ev[k], ev[k + q]
    plus, minus = (fr - di, fi + dr), (fr + di, fi - dr)
    return ((k, (er + sr, ei + si)), (k + 2 * q, (er - sr, ei - si)),
            (k + q, plus if sign > 0 else minus), (k + 3 * q, minus if sign > 0 else plus))


def _fft(xs, sign):
    n = len(xs)
    if n == 1:
        return xs
    if n == 2:
        (ar, ai), (br, bi) = xs
        return [(ar + br, ai + bi), (ar - br, ai - bi)]
    ev, o1, o3 = _fft(xs[0::2], sign), _fft(xs[1::4], sign), _fft(xs[3::4], sign)
    out = dict(pair for k in range(n // 4) for pair in _fft_merge(ev, o1, o3, k, sign))
    return [out[k] for k in range(n)]


def _weave(*streams, drain=True):
    done = [0] * len(streams)
    for _ in range(sum(n for _, n in streams)):
        live = [i for i, (_, n) in enumerate(streams) if done[i] < n]
        i = min(live, key=lambda k: (done[k] + 0.5) / streams[k][1])
        next(streams[i][0], None)
        done[i] += 1
    for gen, _ in streams[0 if drain else 1:]:
        for _ in gen:
            pass


def _skew(gens, gap=1):
    gens, active = list(gens), []
    for step in itertools.count():
        if gens and (step % gap == 0 or not active):
            active.append(gens.pop(0))
        if not active:
            return
        for gen in list(active):
            if next(gen, active) is active:
                active.remove(gen)
            if active or gens:
                yield


def _mean(v):
    return jnp.mean(v, axis=-1, keepdims=True)


def _layernorm(x):
    mu = _mean(x)
    yield
    xc = x - mu
    var = _mean(xc * xc)
    yield
    rstd = lax.rsqrt(var + EPS)
    return xc * rstd, (mu, rstd)


def _layernorm_bwd(x, stats, dn):
    mu, rstd = stats
    n = (x - mu) * rstd
    dmu, proj = _mean(dn), _mean(dn * n)
    yield
    return n, rstd * (dn - dmu - n * proj)


def _fold8(v):
    acc = v[0:8]
    for i in range(1, v.shape[0] // 8):
        acc = acc + v[8 * i:8 * i + 8]
    return acc


def _unpack(p):
    return lax.bitcast_convert_type(p << 16, F32), lax.bitcast_convert_type(p & HI16, F32)


def _pack(lo, hi):
    return pltpu.pack_elementwise([lo, hi], packed_dtype=BF).astype(I32)


def _even_odd(v):
    return _unpack(pltpu.bitcast(v, I32))


def _reverse64(v):
    row = lax.broadcasted_iota(I32, (8, 128), 0)
    odd, upper = (row & 1) == 1, (row & 2) == 2
    out = []
    for i in range(7, -1, -1):
        t = pltpu.roll(v[8 * i:8 * i + 8], 4, 0)
        t = jnp.where(upper, pltpu.roll(t, 2, 0), pltpu.roll(t, 6, 0))
        out.append(jnp.where(odd, pltpu.roll(t, 1, 0), pltpu.roll(t, 7, 0)))
    return jnp.concatenate(out, axis=0)


def _partner(va, vb, special):
    if special:
        return pltpu.roll(_reverse64(va), 1, 0), _reverse64(vb)
    return vb, va


def _slot(f1):
    return (f1 % 2) * 16 + f1 // 2


(S_MODA, S_MODG, S_MODR, S_FD, S_MF, S_WR, S_WI, S_DWR, S_DWI, S_DMA, S_DMB, S_C, S_DC) = range(13)


def _kernel(c_hbm, x_hbm, wr_hbm, wi_hbm, wg_hbm, wu_hbm, wd_hbm, wm_hbm, g_hbm, fd_hbm, mf_hbm,
            out_hbm, dx_hbm, dwr_hbm, dwi_hbm, dwg_hbm, dwu_hbm, dwd_hbm, dc_hbm, dwm_hbm,
            xv, gv, wm, wgu, wd, wr, mod, wi, sums, fd, mf, ybuf, xs, wt, shuffle, av, ln, dx1, stage,
            ah, pt, cb, bgu, bd, dact, q, cv, dcv,
            sem, sem_x, sem_g, sem_w, sem_o, sem_dx, sem_dd, sem_fence):
    cp = pltpu.make_async_copy
    scopes = contextlib.ExitStack()

    def fence():
        pl.semaphore_signal(sem_fence, 1)
        pl.semaphore_wait(sem_fence, 1)

    def phase(name):
        scopes.close()
        fence()
        if name:
            scopes.enter_context(jax.named_scope(name))

    def rows_of(i, n):
        return pl.ds(i * n if isinstance(i, int) else pl.multiple_of(i * n, n), n)

    def half_rows(i, half, n=R):
        start = half * H + i * n
        return pl.ds(start if isinstance(i, int) else pl.multiple_of(start, n), n)

    def x_copy(i, half):
        return cp(x_hbm.at[half_rows(i, half, 256)], xv.at[half_rows(i, half, 256)], sem_x.at[2 * i + half])

    def g_copy(i, half):
        return cp(g_hbm.at[half_rows(i, half, 256)], gv.at[half_rows(i, half, 256)], sem_g.at[2 * i + half])

    def wd_rows(j, half):
        start = half * FH + j * 128
        return pl.ds(start if isinstance(j, int) else pl.multiple_of(start, 128), 128)

    def wd_copy(j, half):
        return cp(wd_hbm.at[wd_rows(j, half)], wd.at[wd_rows(j, half)], sem_dd.at[2 * j + half])

    def wgu_copy(t):
        src = wg_hbm if t < 2 * NJ else wu_hbm
        return cp(src.at[:, pl.ds(128 * (t % (2 * NJ)), 128)], wgu.at[t], sem_w.at[t])

    def mod_copy(lo, hi, s):
        return cp(wm_hbm.at[:, pl.ds(lo, hi - lo)], wm.at[:, pl.ds(lo, hi - lo)], sem.at[s])

    def dmod_copy(lo, hi, s):
        return cp(wm.at[:, pl.ds(lo, hi - lo)], dwm_hbm.at[:, pl.ds(lo, hi - lo)], sem.at[s])

    def out_copy(i, half):
        return cp(stage.at[half_rows(i, half)], out_hbm.at[half_rows(i, half)], sem_o.at[2 * i + half])

    def dx_copy(i, half):
        return cp(stage.at[half_rows(i, half, 256)], dx_hbm.at[half_rows(i, half, 256)], sem_dx.at[2 * i + half])

    def dwgu_copy(dst, t, half):
        j = t % NJ + NJ * half
        slot = (t // NJ) * 2 * NJ + j
        return cp(wgu.at[slot], dst.at[:, rows_of(j, 128)], sem_w.at[slot])

    def dwd_copy(j, half):
        return cp(wd.at[wd_rows(j, half)], dwd_hbm.at[wd_rows(j, half)], sem_dd.at[2 * j + half])

    in_copies = dict(
        c=cp(c_hbm, cv, sem.at[S_C]),
        moda=mod_copy(0, 2 * D, S_MODA), modr=mod_copy(2 * D, 5 * D, S_MODR), modg=mod_copy(5 * D, 6 * D, S_MODG),
        fd=cp(fd_hbm, fd, sem.at[S_FD]), mf=cp(mf_hbm, mf, sem.at[S_MF]),
        wr=cp(wr_hbm, wr, sem.at[S_WR]), wi=cp(wi_hbm, wi, sem.at[S_WI]))

    fd, mf, ah, pt, cb, bd = [_Packed(ref) for ref in (fd, mf, ah, pt, cb, bd)]

    def both(copy, i, wait=False):
        for half in range(2):
            copy(i, half).wait() if wait else copy(i, half).start()

    in_copies["c"].start()
    both(wd_copy, 0)
    in_copies["modg"].start()
    both(g_copy, 0)

    phase("s00_start")
    in_copies["c"].wait()
    cf = cv[...].astype(F32)
    sig = 1.0 / (1.0 + jnp.exp(-cf))
    silu = (cf * sig).astype(BF)
    silu16 = jnp.broadcast_to(silu, (16, D))

    def modulation(k):
        mod[k] = _dot(silu16, wm[:, k * D:(k + 1) * D])[0:8]

    def mod_row(k):
        return mod[k, 0:1, :]

    def slab_rows(b, s, half=0):
        start = half * H + 64 * b + 16 * s
        return pl.ds(start if isinstance(b, int) else pl.multiple_of(start, 16), 16)

    def slab(ref, b, s):
        return jnp.concatenate([ref[slab_rows(b, s, 0), :], ref[slab_rows(b, s, 1), :]], axis=0)

    def put_slab(ref, b, s, v):
        ref[slab_rows(b, s, 0), :] = v[:16]
        ref[slab_rows(b, s, 1), :] = v[16:]

    def pace(v, *refs):
        for ref in refs:
            n = 16 if ref.dtype == BF else 8
            piece = v[:n, :128]
            piece = piece.astype(BF) if n == 16 else lax.bitcast_convert_type(piece, ref.dtype)
            last = tuple(d - 1 for d in ref.shape[:-2])
            ref[last + (slice(ref.shape[-2] - n, ref.shape[-2]), slice(0, 128))] = piece

    paced = []

    def put_stats(k, b, s, stats):
        for t, v in enumerate(stats):
            put_slab(ln.at[2 * k + t], b, s, jnp.broadcast_to(v, (32, 128)))

    def get_stats(k, b, s):
        return [jnp.concatenate([slab(ln.at[2 * k + t], b, s)] * (D // 128), axis=1) for t in range(2)]

    def dft_operands(h, three=False):
        rows = (h[:16] + h[16:], h[:16] - h[16:])
        even = [v[:, :256] + v[:, 256:] for v in rows]
        odd = [v[:, :256] - v[:, 256:] for v in rows]
        return ([(v[:, :128] + v[:, 128:]).astype(BF) for v in even],
                [(v[:, :128] - v[:, 128:]).astype(BF) for v in even],
                *([[v[:, :128].astype(BF) for v in odd], [v[:, 128:].astype(BF) for v in odd],
                   [(v[:, :128] + v[:, 128:]).astype(BF) for v in odd]] if three else [[v.astype(BF) for v in odd]]))

    lane = lax.broadcasted_iota(I32, (128, 128), 1)
    low_lanes, odd_sign = lane < 64, jnp.where((lane & 1) == 1, 1.0, -1.0)

    def model_dft(slabs, b, delay):
        for _ in range(delay):
            yield
        v0, v2, *vo = [jnp.concatenate([v[k][0] for v in slabs] + [v[k][1] for v in slabs], axis=0)
                       for k in range(len(slabs[0]))]
        y0, y2 = _dot(v0, fd[0, 0:128, 0:128]), _dot(v2, fd[0, 0:128, 128:256])
        planes = [(jnp.where(low_lanes, y0, y2), pltpu.roll(jnp.where(low_lanes, y2, y0), 64, 1))]
        yield
        if len(vo) == 1:
            yo = _dot(vo[0], fd[1])
            planes.append((yo[:, :128], yo[:, 128:]))
        else:
            shared = _dot(vo[2], fd[2, 0:128, 0:128])
            planes.append((shared - _dot(vo[1], fd[2, 0:128, 128:256]),
                           (shared + _dot(vo[0], fd[2, 128:256, 0:128])) * odd_sign))
        for k, (re, im) in enumerate(planes):
            yield
            lanes = slice(128 * k, 128 * k + 128)
            ybuf[b, 0:64, lanes], ybuf[b, 64:128, lanes] = re[:64], im[:64]
            ybuf[16 + b, 0:64, lanes], ybuf[16 + b, 64:128, lanes] = re[64:], im[64:]
        yield

    def model_idft(b, parts):
        def plane(rows, lanes):
            return jnp.concatenate([ybuf[b, rows, lanes], ybuf[16 + b, rows, lanes]], axis=0)
        re, im = plane(slice(0, 64), slice(0, 128)), pltpu.roll(plane(slice(64, 128), slice(0, 128)), 64, 1)
        p0 = _dot(jnp.where(low_lanes, re, im).astype(BF), fd[0, 0:128, 0:128], NT)
        p2 = _dot(jnp.where(low_lanes, im, re).astype(BF), fd[0, 0:128, 128:256], NT)
        parts.append(jnp.concatenate([p0 + p2, p0 - p2], axis=1))
        yield
        v = jnp.concatenate([plane(slice(0, 64), slice(128, 256)), plane(slice(64, 128), slice(128, 256))], axis=1)
        parts.append(_dot(v.astype(BF), fd[1], NT))

    def idft_slab(parts, s):
        p, o = [jnp.concatenate([v[16 * s:16 * s + 16], v[64 + 16 * s:80 + 16 * s]], axis=0) for v in parts]
        y = jnp.concatenate([p + o, p - o], axis=1)
        return jnp.concatenate([y[:16] + y[16:], y[:16] - y[16:]], axis=0)

    def seq_fft(sign):
        for g in range(8):
            re, im = pl.ds(8 * g, 8), pl.ds(64 + 8 * g, 8)
            for lanes in (slice(0, 128), slice(128, 256)):
                for odd in range(2):
                    z = [(ybuf[16 * odd + b, re, lanes], ybuf[16 * odd + b, im, lanes]) for b in range(16)]
                    yield
                    if odd and sign < 0:
                        z = [_twiddle(v, b, 32, sign) for b, v in enumerate(z)]
                    ev = _fft(z[0::2], sign)
                    yield
                    o1, o3 = _fft(z[1::4], sign), _fft(z[3::4], sign)
                    yield
                    for k in range(4):
                        for b, v in _fft_merge(ev, o1, o3, k, sign):
                            if odd and sign > 0:
                                v = _twiddle(v, b, 32, sign)
                            ybuf[16 * odd + b, re, lanes] = v[0]
                            ybuf[16 * odd + b, im, lanes] = v[1]
                        if k % 2:
                            yield

    lane0 = lax.broadcasted_iota(I32, (64, 128), 1) == 0

    def residue(f1):
        return pl.ds(PITCH * f1, 64)

    def residue_octet(f0, a):
        return pl.ds(PITCH * 8 * a + (f0 if a < 2 else 63 - f0), 8, stride=PITCH)

    def bd_prep(js):
        for j in js:
            for o in range(0, 128, 32):
                lo, hi = pl.ds(128 * j + o, 32), pl.ds(FH + 128 * j + o, 32)
                w = wd[lo, 0:256], wd[lo, 256:512], wd[hi, 0:256], wd[hi, 256:512]
                yield
                even, odd = [_comb_b(*v) for v in zip(*map(_even_odd, w))]
                for r in range(7):
                    bd[r, lo, :] = _pack(even[r], odd[r])

    def cb_prep(i):
        for o in range(0, 256, 32):
            lo, hi = pl.ds(256 * i + o, 32), pl.ds(H + 256 * i + o, 32)
            parts = []
            for dlo, dhi in zip(_even_odd(gv[lo, :]), _even_odd(gv[hi, :])):
                dlo, dhi = dlo * mod_row(5), dhi * mod_row(5)
                parts.append(_comb_dc(dlo[:, :256], dlo[:, 256:], dhi[:, :256], dhi[:, 256:]))
            for r in range(7):
                cb[r, lo, :] = _pack(parts[0][r], parts[1][r])

    piece = [128]

    def dact_stream():
        for j in range(NJ):
            o = 0
            while o < H:
                m = piece[0] if o % 128 == 0 else 64
                prods = []
                for r in range(7):
                    prods.append(_dot(cb[r, o:o + m], bd[r, 128 * j:128 * j + 128], NT))
                    for _ in range(m // 64):
                        yield
                parts = _comb_da(prods)
                dact[j, 0, o:o + m] = _pack(parts[0], parts[1])
                dact[j, 1, o:o + m] = _pack(parts[2], parts[3])
                o += m
    filler = dact_stream()

    def fill(n, stream, steps, rows=128):
        piece[0] = rows
        _weave((filler, 4 * n), (stream, steps), drain=False)

    both(wd_copy, 0, wait=True)
    both(g_copy, 1)
    _weave((bd_prep([0]), 4))
    in_copies["modg"].wait()
    modulation(5)
    for i in range(4):
        both(g_copy, i, wait=True)
        if i < 2:
            both(g_copy, i + 2)
        elif i == 2:
            both(wd_copy, 1)
            in_copies["moda"].start()
        else:
            both(wd_copy, 2)
            in_copies["fd"].start()
            both(x_copy, 0)
        cb_prep(i)
        _weave((filler, 28), drain=False)
    phase("s01_u0")
    both(wd_copy, 1, wait=True)
    for i in range(1, 4):
        both(x_copy, i)
    _weave((bd_prep([1]), 4))
    _weave((filler, 4 * 28), drain=False)
    both(wd_copy, 2, wait=True)
    for j in range(3, NJ):
        both(wd_copy, j)
    for name in ("wr", "wi", "mf"):
        in_copies[name].start()
    _weave((bd_prep([2]), 4))
    _weave((filler, 4 * 7), drain=False)

    phase("s02_p1a")
    in_copies["moda"].wait()
    in_copies["fd"].wait()
    modulation(0)
    modulation(1)

    def p1a_slab(b, s, out):
        n, stats = yield from _layernorm(slab(xv, b, s).astype(F32))
        put_stats(0, b, s, stats)
        out.append(dft_operands(n * (1.0 + mod_row(1)) + mod_row(0)))

    def p1a(bs):
        gens = []
        for b in bs:
            out = []
            gens += [p1a_slab(b, s, out) for s in range(4)] + [model_dft(out, b, 1)]
        return _skew(gens)
    for i in range(2):
        both(x_copy, 2 * i, wait=True)
        both(x_copy, 2 * i + 1, wait=True)
        fill(6, p1a(range(8 * i, 8 * i + 8)), 8 * 17)
    in_copies["modr"].start()
    for t in range(4 * NJ):
        wgu_copy(t).start()
    for j in range(3, NJ):
        both(wd_copy, j, wait=True)
    fill(6, bd_prep(range(3, NJ)), 16, 64)

    phase("s03_p1b")
    fill(20, seq_fft(-1), 160, 64)

    phase("s04_wprep")
    for name in ("wr", "wi", "mf"):
        in_copies[name].wait()

    def filter_prep():
        for t in range(16):
            cols = slice(128 * t, 128 * t + 128)
            r32 = pltpu.bitcast(wr[0:256, cols], I32)
            i32 = pltpu.bitcast(wi[0:256, cols], I32)
            nyq = _pack(wr[256:257, cols].astype(F32), wi[256:257, cols].astype(F32))
            shuffle[t, 0:128] = (r32 & 0xFFFF) | (i32 << 16)
            even = jnp.concatenate([shuffle[t, pl.ds(o, 64, stride=2), :] for o in range(2)], axis=0)
            tiles = (even, lax.shift_right_logical(r32, 16) | (i32 & HI16),
                     jnp.broadcast_to(nyq, (128, 128)))
            for k, tile in enumerate(tiles):
                yield
                tile = tile.T
                for v in range(16):
                    wt[k, residue_octet(4 * t + v // 4, v % 4), :] = tile[8 * v:8 * v + 8]
        for p in range(16):
            f1s = (p, 32 - p) if p else (0, 16)
            w0 = [wt[0, residue(f1), :] for f1 in f1s]
            wn = [wt[2, residue(f1), :] for f1 in f1s]
            yield
            w0m, wnm = _partner(w0[0], w0[1], p == 0), _partner(wn[0], wn[1], p == 0)
            for k, f1 in enumerate(f1s):
                if k == 0 or p == 0:
                    (ar, ai), (br, bi) = _unpack(w0[k]), _unpack(w0m[k])
                    (cr, ci), (dr, di) = _unpack(wn[k]), _unpack(wnm[k])
                    s0r, s0i, snr, sni = ar + br, ai - bi, cr + dr, ci - di
                    alpha = _pack(0.125 * (s0r + snr), 0.125 * (s0i + sni))
                    beta = _pack(0.125 * (s0r - snr), 0.125 * (s0i - sni))
                else:
                    alpha, beta = alpha ^ SIGN, beta ^ SIGN
                wt[0, residue(f1), :] = jnp.where(lane0, alpha, w0[k])
                wt[2, residue(f1), :] = jnp.where(lane0, beta, 0)
    fill(22, filter_prep(), 64, 64)

    phase("s05_p1c")

    def spectral_pair(p, backward, special=False):
        f1s = (0, 16) if special else (p, 32 - p)
        z = []
        for f1 in f1s:
            z.append(_dot(mf[0, f1], ybuf[_slot(f1)].astype(BF)))
            yield
        neg_r = _partner(z[0][0:64, 0:128], z[1][0:64, 0:128], special)
        neg_i = _partner(z[0][64:128, 0:128], z[1][64:128, 0:128], special)
        prod = [([], []), ([], [])]
        for o in range(0, 64, 16):
            for k, f1 in enumerate(f1s):
                rows = pl.ds(PITCH * f1 + o, 16)
                er, orr = z[k][o:o + 16, :128], z[k][o:o + 16, 128:]
                ei, oi = z[k][64 + o:80 + o, :128], z[k][64 + o:80 + o, 128:]
                mr, mi = neg_r[k][o:o + 16], neg_i[k][o:o + 16]
                (ar, ai), (cr, ci), (br, bi) = [_unpack(wt[t, rows, :]) for t in range(3)]
                edge = lane0[:16]
                if backward:
                    pe = (ar * er + ai * ei + (br * mr - bi * mi), ar * ei - ai * er - (br * mi + bi * mr))
                    po = (cr * orr + ci * oi, cr * oi - ci * orr)
                    grads = ((jnp.where(edge, er + mr, er), jnp.where(edge, ei - mi, ei)), (orr, oi), (er - mr, ei + mi))
                    for t, (gr, gi) in enumerate(grads):
                        xr, xi = _unpack(xs[f1, t, o:o + 16])
                        wt[t, rows, :] = _pack(gr * xr + gi * xi, gi * xr - gr * xi)
                else:
                    pe = (ar * er - ai * ei + (br * mr + bi * mi), ar * ei + ai * er + (bi * mr - br * mi))
                    po = (cr * orr - ci * oi, cr * oi + ci * orr)
                    xs[f1, 0, o:o + 16] = _pack(jnp.where(edge, 0.125 * (er + mr), er),
                                                jnp.where(edge, 0.125 * (ei - mi), ei))
                    xs[f1, 1, o:o + 16] = _pack(orr, oi)
                    xs[f1, 2, o:o + 16] = _pack(0.125 * (er - mr), 0.125 * (ei + mi))
                for part in range(2):
                    prod[k][part].append(jnp.concatenate([pe[part], po[part]], axis=1).astype(BF))
                yield
        for k, f1 in enumerate(f1s):
            y = _dot(mf[1, f1], jnp.concatenate(prod[k][0] + prod[k][1], axis=0))
            yield
            ybuf[_slot(f1)] = y
    fill(25, _skew([spectral_pair(p, False, p == 0) for p in range(16)], 6), 16 * 13)

    phase("s06_p1d")
    fill(20, seq_fft(1), 160, 64)

    phase("s07_bgu")
    in_copies["modr"].wait()
    for t in range(4 * NJ):
        wgu_copy(t).wait()
    for k in (2, 3, 4):
        modulation(k)

    def bgu_prep():
        for t in range(2 * NJ):
            lo = (t // NJ) * 2 * NJ + t % NJ
            for o in range(0, 256, 64):
                a, b = slice(o, o + 64), slice(256 + o, 256 + o + 64)
                w = wgu[lo, a], wgu[lo + NJ, a], wgu[lo, b], wgu[lo + NJ, b]
                yield
                for r, part in enumerate(_comb_b(*[v.astype(F32) for v in w])):
                    if r not in (1, 4):
                        bgu[t, r, a] = part.astype(BF)

    def bgu_tile(t, r):
        lo = (t // NJ) * 2 * NJ + t % NJ
        return wgu[lo, 0:256] if r == 1 else wgu[lo + NJ, 256:512] if r == 4 else bgu[t, r]
    _weave((bgu_prep(), 8 * NJ))

    phase("s08_stage0")

    def residual1(x, a):
        return x.astype(F32) + (SCALE * mod_row(2)) * a

    def stage0_slab(b, s, parts):
        x = slab(xv, b, s)
        yield
        a = idft_slab(parts, s)
        av[slab_rows(b, s), :] = _pack(a[:16], a[16:])
        n, stats = yield from _layernorm(residual1(x, a))
        put_stats(1, b, s, stats)
        h = n * (1.0 + mod_row(4)) + mod_row(3)
        yield
        for r, part in enumerate(_comb_a(h[:16, :256], h[:16, 256:], h[16:, :256], h[16:, 256:])):
            ah[r, slab_rows(b, s), :] = part.astype(BF)

    def stage0():
        gens = []
        for b in range(16):
            parts = []
            gens += [model_idft(b, parts)] + [stage0_slab(b, s, parts) for s in range(4)]
        return _skew(gens)
    piece[0] = 128
    _weave((filler, 4 * 28), (stage0(), 16 * 22))

    sums[...] = jnp.zeros(sums.shape, F32)

    def gate_up(i, j):
        return [_dot(ah[r, rows_of(i, R), :], jnp.concatenate([bgu_tile(j, r), bgu_tile(NJ + j, r)], axis=1))
                for r in range(7)]

    def geglu_chunk(i, j, prods):
        rows = rows_of(i, R)
        da = _unpack(dact[j, 0, rows, :]) + _unpack(dact[j, 1, rows, :])
        res = [_geglu(gu[:, :128], gu[:, 128:], da[k]) for k, gu in enumerate(_comb_c(prods))]
        for t, parts in ((2 * NJ + j, _comb_a(*[v[0] for v in res])),
                         (j, _comb_dc(*[v[1] for v in res])),
                         (NJ + j, _comb_dc(*[v[2] for v in res]))):
            for r in range(7):
                q[t, r, rows, :] = parts[r].astype(BF)

    def d_h2(i, r, tiles):
        return _dot(jnp.concatenate([q[t, r, rows_of(i, R), :] for t in tiles], axis=1),
                    jnp.concatenate([bgu_tile(t, r) for t in tiles], axis=1), NT)

    def ffn_step(i, _):
        early = [t for t in range(2 * NJ) if t % NJ != NJ - 1]
        prods = gate_up(i, 0)
        for j in range(NJ - 1):
            nxt = gate_up(i, j + 1)
            geglu_chunk(i, j, prods)
            prods = nxt
        dh0 = d_h2(i, 0, early)
        geglu_chunk(i, NJ - 1, prods)
        rows = rows_of(i, R)
        b = _comb_c([_dot(jnp.concatenate([q[2 * NJ + j, r, rows, :] for j in range(NJ)], axis=1), bd[r])
                     for r in range(7)])
        dh = {0: dh0 + d_h2(i, 0, (NJ - 1, 2 * NJ - 1))}
        a = _unpack(av[half_rows(i, 0), :])
        for half in range(2):
            out_rows = half_rows(i, half)
            bh = jnp.concatenate([b[2 * half], b[2 * half + 1]], axis=1)
            stage[out_rows, :] = (residual1(xv[out_rows, :], a[half]) + mod_row(5) * bh).astype(BF)
            sums[5] += _fold8(gv[out_rows, :].astype(F32) * bh)
        for r in (1, 2, 4, 5, 6):
            dh[r] = d_h2(i, r, range(2 * NJ))
        for r in range(7):
            pt[0, r, i] = ah[r, rows, :].T
            pt[1, r, i] = cb[r, rows, :].T
        lo, hi = half_rows(i, 0), half_rows(i, 1)
        dx1[lo, 0:256] = dh[0] + dh[2] + dh[4] - dh[5]
        dx1[lo, 256:512] = dh[4] + dh[6]
        dx1[hi, 0:256] = dh[1] + dh[5]
        dx1[hi, 256:512] = (dh[0] + dh[1] - dh[6]) + d_h2(i, 3, range(2 * NJ))
        both(out_copy, i)
    phase("s11_ffn")
    lax.fori_loop(0, H // R, ffn_step, None)

    def wgrad(side, t, store, m):
        for o in range(0, 256, m):
            d = {}
            for r in (0, 2, 3, 5, 6, 1, 4):
                acc = None
                for i in range(0, H // R, 2):
                    lhs = jnp.concatenate([pt[side, r, i, o:o + m], pt[side, r, i + 1, o:o + m]], axis=1)
                    part = _dot(lhs, q[t, r, R * i:R * i + 2 * R])
                    acc = part if acc is None else acc + part
                    for _ in range(m // 64):
                        yield
                pace(acc, *paced)
                d[r] = acc
                if r == 6:
                    store(o, 1, d[2] + d[5])
                    store(o, 2, d[3] + d[6])
                elif r == 1:
                    store(o, 0, (d[0] - d[3] + d[5]) + d[1])
                elif r == 4:
                    store(o, 3, (d[0] - d[2] + d[6]) + d[4])

    def wgrad_gate_up(t, m=64):
        lo = (t // NJ) * 2 * NJ + t % NJ

        def store(o, k, d):
            start = 256 * (k // 2) + o
            wgu[lo + NJ * (k % 2), start:start + m] = d.astype(BF)
        return wgrad(0, t, store, m)

    def gate_up_send(dst, t):
        for half in range(2):
            dwgu_copy(dst, t, half).start()

    def wgrad_down(j):
        def store(o, k, d):
            col = 256 * (k % 2) + o
            wd[wd_rows(j, k // 2), col:col + 128] = d.T.astype(BF)
        return wgrad(1, 2 * NJ + j, store, 128)

    phase("s13_stagec")

    def stage_c_slab(b, s, acc, out):
        a = jnp.concatenate(_unpack(av[slab_rows(b, s), :]), axis=0)
        dh = slab(dx1, b, s)
        n, d = yield from _layernorm_bwd(residual1(slab(xv, b, s), a), get_stats(1, b, s), dh * (1.0 + mod_row(4)))
        d = d + slab(gv, b, s).astype(F32)
        put_slab(dx1, b, s, d)
        pace(d, xv, gv, av)
        yield
        acc[:] = [acc[0] + _fold8(d * a), acc[1] + _fold8(dh), acc[2] + _fold8(dh * n)]
        yield
        out.append(dft_operands(d * (SCALE * mod_row(2)), three=True))

    def stage_c_rows(bs):
        acc, gens = [sums[k] for k in (2, 3, 4)], []
        for b in bs:
            out = []
            gens += [stage_c_slab(b, s, acc, out) for s in range(4)] + [model_dft(out, b, 2)]
        yield from _skew(gens)
        for k, v in zip((2, 3, 4), acc):
            sums[k] = v

    paced[:] = [xv]

    def stage_c(i, _):
        tiles = (2 * i, 2 * i + 1, NJ + 2 * i, NJ + 2 * i + 1)
        _weave((itertools.chain(*[wgrad_gate_up(t, 128) for t in tiles]), 448),
               (stage_c_rows([8 * i + u for u in range(8)]), 8 * 23))
        for t, dst in zip(tiles, (dwg_hbm, dwg_hbm, dwu_hbm, dwu_hbm)):
            gate_up_send(dst, t)
    lax.fori_loop(0, 2, stage_c, None)

    phase("s14_p3b")
    paced[:] = [ybuf]
    _weave((wgrad_gate_up(4), 112), (seq_fft(-1), 160))
    gate_up_send(dwg_hbm, 4)

    phase("s15_p3c")

    tiles = (NJ + 4, NJ + 5, NJ + 6, 5)
    paced[:] = []
    _weave((itertools.chain(*[wgrad_gate_up(t, 128) for t in tiles]), 448),
           (_skew([spectral_pair(p, True, p == 0) for p in range(16)], 3), 16 * 13))
    for t in tiles:
        gate_up_send(dwg_hbm if t < NJ else dwu_hbm, t)

    phase("s16_p3d")
    paced[:] = [ybuf]
    _weave((wgrad_gate_up(6), 112), (seq_fft(1), 160))
    gate_up_send(dwg_hbm, 6)

    phase("s17_dw")

    def filter_grad_out():
        for t in range(16):
            cols = slice(128 * t, 128 * t + 128)
            tiles = []
            for k in range(3):
                tiles.append(jnp.concatenate(
                    [wt[k, residue_octet(4 * t + v // 4, v % 4), :] for v in range(16)], axis=0).T)
                yield
            ev, od, nyq = tiles
            for o in range(2):
                shuffle[t, pl.ds(o, 64, stride=2), :] = ev[64 * o:64 * o + 64]
            ev = shuffle[t, 0:128]
            wr[0:256, cols] = pltpu.bitcast((ev & 0xFFFF) | (od << 16), BF)
            wi[0:256, cols] = pltpu.bitcast(lax.shift_right_logical(ev, 16) | (od & HI16), BF)
            nr, ni = _unpack(nyq[0:1])
            wr[256:257, cols] = nr.astype(BF)
            wi[256:257, cols] = ni.astype(BF)
    paced[:] = []

    def modulation_bwd(ks):
        silu_col = jnp.broadcast_to(silu.astype(F32), (128, D)).T
        row = lax.broadcasted_iota(I32, (16, D), 0)
        for k in ks:
            dm = jnp.sum(sums[k], axis=0, keepdims=True) * (SCALE if k == 2 else 1.0)
            hi = dm.astype(BF).astype(F32)
            lhs = jnp.where(row == 0, hi, jnp.where(row == 1, dm - hi, 0.0)).astype(BF)
            mod[3] += _dot(lhs, wm[:, k * D:(k + 1) * D], NT)[0:8]
            yield
            for t in range(D // 128):
                cols = slice(k * D + 128 * t, k * D + 128 * t + 128)
                wm[:, cols] = (silu_col * dm[:, 128 * t:128 * t + 128]).astype(BF)
                yield

    mod[3] = jnp.zeros((8, D), F32)
    _weave((itertools.chain(wgrad_down(0), wgrad_down(1)), 224), (filter_grad_out(), 48),
           (modulation_bwd((2, 3, 4, 5)), 20))
    both(dwd_copy, 0)
    both(dwd_copy, 1)
    dmod_copy(2 * D, 6 * D, S_DMB).start()
    dwr_copy, dwi_copy = cp(wr, dwr_hbm, sem.at[S_DWR]), cp(wi, dwi_hbm, sem.at[S_DWI])
    dwr_copy.start()
    dwi_copy.start()
    for i in range(H // R):
        both(out_copy, i, wait=True)

    phase("s18_p3e")

    def p3e_slab(b, s, acc, parts):
        x = slab(xv, b, s)
        yield
        dh = idft_slab(parts, s)
        n, d = yield from _layernorm_bwd(x.astype(F32), get_stats(0, b, s), dh * (1.0 + mod_row(1)))
        d = d + slab(dx1, b, s)
        put_slab(stage, b, s, d.astype(BF))
        pace(d, xv)
        dx1[slab_rows(b, s), 0:128] = d[:16, :128]
        yield
        acc[:] = [acc[0] + _fold8(dh), acc[1] + _fold8(dh * n)]

    def send_dx(i):
        for _ in range(4):
            yield
        both(dx_copy, i)

    def p3e_rows():
        acc, gens = [sums[0], sums[1]], []
        for b in range(16):
            parts = []
            gens += [model_idft(b, parts)] + [p3e_slab(b, s, acc, parts) for s in range(4)]
            if b % 4 == 3:
                gens.append(send_dx(b // 4))
        yield from _skew(gens)
        sums[0], sums[1] = acc

    paced[:] = [xv]
    _weave((itertools.chain(*[wgrad_down(j) for j in range(2, 6)]), 448), (p3e_rows(), 16 * 18 + 20))
    for j in range(2, 6):
        both(dwd_copy, j)
    paced[:] = []

    phase("s19_tail")
    last = wgrad_down(6)
    _weave((last, 32), (modulation_bwd((0, 1)), 10), drain=False)
    dmod_copy(0, 2 * D, S_DMA).start()
    dcv[...] = ((mod[3, 0:1] + mod[3, 1:2]) * (sig * (1.0 + cf * (1.0 - sig)))).astype(BF)
    dc_copy = cp(dcv, dc_hbm, sem.at[S_DC])
    dc_copy.start()
    _weave((last, 80))
    both(dwd_copy, 6)

    phase("s20_wait")
    for t in range(2 * NJ):
        for half in range(2):
            dwgu_copy(dwg_hbm if t < NJ else dwu_hbm, t, half).wait()
    dc_copy.wait()
    dwr_copy.wait()
    dwi_copy.wait()
    for i in range(4):
        both(dx_copy, i, wait=True)
    dmod_copy(2 * D, 6 * D, S_DMB).wait()
    dmod_copy(0, 2 * D, S_DMA).wait()
    for j in range(NJ):
        both(dwd_copy, j, wait=True)
    phase(None)


@jax.jit
def pallas_adaLN_cond__spectral_gfnet__geglu_ffn__prompt_kernel(
    A_x: jax.Array,
    A_w_r: jax.Array,
    A_w_i: jax.Array,
    B_x: jax.Array,
    B_w_gate: jax.Array,
    B_w_up: jax.Array,
    B_w_down: jax.Array,
    c: jax.Array,
    w_mod: jax.Array,
    grad_out: jax.Array,
):
    del B_x
    kf = D // 2 + 1
    hbm = pl.BlockSpec(memory_space=pltpu.MemorySpace.HBM)
    sds = jax.ShapeDtypeStruct
    dma = pltpu.SemaphoreType.DMA
    out, dx, dwr, dwi, dwg, dwu, dwd, dc, dwm = pl.pallas_call(
        _kernel,
        in_specs=[hbm] * 11,
        out_specs=[hbm] * 9,
        out_shape=[sds((S, D), BF), sds((S, D), BF), sds((kf, S), BF), sds((kf, S), BF),
                   sds((D, F), BF), sds((D, F), BF), sds((F, D), BF), sds((1, D), BF), sds((D, 6 * D), BF)],
        scratch_shapes=[
            pltpu.VMEM((S + 128, D), BF),
            pltpu.VMEM((S + 128, D), BF),
            pltpu.VMEM((D, 6 * D), BF),
            pltpu.VMEM((4 * NJ, D, 128), BF),
            pltpu.VMEM((F, D), BF),
            pltpu.VMEM((kf, S), BF),
            pltpu.VMEM((6, 8, D), F32),
            pltpu.VMEM((kf, S), BF),
            pltpu.VMEM((6, 8, D), F32),
            _packed(3, 256, 256),
            _packed(2, 32, 128, 128),
            pltpu.VMEM((33, 128, 256), F32),
            pltpu.VMEM((32, 3, 64, 128), I32),
            pltpu.VMEM((3, 36 * 64, 128), I32),
            pltpu.VMEM((16, 136, 128), I32),
            pltpu.VMEM((H + 64, D), I32),
            pltpu.VMEM((4, S, 128), F32),
            pltpu.VMEM((S, D), F32),
            pltpu.VMEM((S, D), BF),
            _packed(7, H, 256),
            _packed(2, 7, H // R, 256, R),
            _packed(7, H, 256),
            pltpu.VMEM((2 * NJ, 7, 256, 128), BF),
            _packed(8, FH, 256),
            pltpu.VMEM((NJ, 2, H, 128), I32),
            pltpu.VMEM((3 * NJ, 7, H, 128), BF),
            pltpu.VMEM((1, D), BF),
            pltpu.VMEM((1, D), BF),
            dma((13,)), dma((8,)), dma((8,)), dma((4 * NJ,)), dma((2 * H // R,)), dma((8,)), dma((2 * NJ,)),
            pltpu.SemaphoreType.REGULAR,
        ],
        compiler_params=pltpu.CompilerParams(vmem_limit_bytes=126 * 1024 * 1024),
    )(c, A_x.reshape(S, D), A_w_r.T, A_w_i.T, B_w_gate, B_w_up, B_w_down, w_mod,
      grad_out.reshape(S, D), _FD, _MF)
    return (out.reshape(1, S, D), dx.reshape(1, S, D), dwr.T, dwi.T, dwg, dwu, dwd, dc, dwm)
```
